```python
import jax
import jax.numpy as jnp

def _softmax(x, axis=-1):
    return jax.nn.softmax(x, axis=axis)

def _gelu(x):
    return jax.nn.gelu(x, approximate=True)

def _silu(x):
    return jax.nn.silu(x)

def _sigmoid(x):
    return jax.nn.sigmoid(x)

def _layernorm(x, axis=-1, eps=1e-05):
    m = jnp.mean(x, axis=axis, keepdims=True)
    v = jnp.var(x, axis=axis, keepdims=True)
    return (x - m) / jnp.sqrt(v + eps)

def _scatter_add(tgt, idx, src, axis=0):
    return tgt.at[idx].add(src)

def _segment_sum(src, seg, n):
    return jax.ops.segment_sum(src, seg, n)

class _Rng:

    def __init__(self, key):
        self._k = key

    def _next(self):
        self._k, sub = jax.random.split(self._k)
        return sub

    def normal(self, shape):
        return jax.random.normal(self._next(), shape, dtype=jnp.bfloat16)

    def randint(self, lo, hi, shape):
        return jax.random.randint(self._next(), shape, lo, hi, dtype=jnp.int32)

    def uniform(self, shape, lo=0.0, hi=1.0):
        return jax.random.uniform(self._next(), shape, jnp.bfloat16, lo, hi)

    def permutation(self, n):
        return jax.random.permutation(self._next(), n)
kernel_name = 'adaLN_cond__compressed_kv_cla__glu_gated_geglu__decode'

def setup_inputs():
    _rng = _Rng(jax.random.key(int.from_bytes(__import__("os").urandom(4), "little")))
    _w = lambda a: (lambda t: t.astype(jnp.bfloat16) if jnp.issubdtype(t.dtype, jnp.floating) else t)(jnp.asarray(a))

    def _A_setup():
        B, H, Sq, Sk, D, M = (1, 32, 1, 32768, 128, 512)
        Dc = 4 * D
        return {'x': _w((lambda *s: _rng.normal(s) * 0.05)(B, Sq, M)), 'c_kv': _w((lambda *s: _rng.normal(s) * 0.05)(B, Sk, Dc)), 'w_q': _w((lambda *s: _rng.normal(s) * 0.05)(M, H, D) * M ** (-0.5)), 'w_uk': _w((lambda *s: _rng.normal(s) * 0.05)(Dc, H, D) * Dc ** (-0.5)), 'w_uv': _w((lambda *s: _rng.normal(s) * 0.05)(Dc, H, D) * Dc ** (-0.5)), 'w_o': _w((lambda *s: _rng.normal(s) * 0.05)(H, D, M) * (H * D) ** (-0.5))}
    _A_in = _A_setup()

    def _B_setup():
        B, S, Dm, Df = (1, 1, 512, 1792)
        return {'x': _w((lambda *s: _rng.normal(s) * 0.05)(B, S, Dm)), 'w_gate': _w((lambda *s: _rng.normal(s) * 0.05)(Dm, Df) * Dm ** (-0.5)), 'w_up': _w((lambda *s: _rng.normal(s) * 0.05)(Dm, Df) * Dm ** (-0.5)), 'w_down': _w((lambda *s: _rng.normal(s) * 0.05)(Df, Dm) * Df ** (-0.5))}
    _B_in = _B_setup()
    return {'A_x': _A_in['x'], 'A_c_kv': _A_in['c_kv'], 'A_w_q': _A_in['w_q'], 'A_w_uk': _A_in['w_uk'], 'A_w_uv': _A_in['w_uv'], 'A_w_o': _A_in['w_o'], 'B_x': _B_in['x'], 'B_w_gate': _B_in['w_gate'], 'B_w_up': _B_in['w_up'], 'B_w_down': _B_in['w_down'], 'c': _w((lambda *s: _rng.normal(s) * 0.05)(1, 512)), 'w_mod': _w((lambda *s: _rng.normal(s) * 0.05)(512, 6 * 512) * 512 ** (-0.5))}

def reference(A_x, A_c_kv, A_w_q, A_w_uk, A_w_uv, A_w_o, B_x, B_w_gate, B_w_up, B_w_down, c, w_mod):

    def _A_ref(x, c_kv, w_q, w_uk, w_uv, w_o):
        B, Sq, M = (x.shape[0], x.shape[1], x.shape[2])
        Sk = c_kv.shape[1]
        H, D = (w_q.shape[1], w_q.shape[2])
        q = jnp.einsum('bqm,mhd->bhqd', x, w_q)
        k = jnp.einsum('bkc,chd->bhkd', c_kv, w_uk)
        v = jnp.einsum('bkc,chd->bhkd', c_kv, w_uv)
        scores = jnp.einsum('bhqd,bhkd->bhqk', q, k) * D ** (-0.5)
        off = Sk - Sq
        qi = jnp.arange(Sq)[:, None]
        kj = jnp.arange(Sk)[None, :]
        cmask = kj <= qi + off
        scores = jnp.where(cmask[None, None], scores, -1000000000.0)
        p = _softmax(scores, axis=-1)
        ctx = jnp.einsum('bhqk,bhkd->bhqd', p, v)
        return jnp.einsum('bhqd,hdm->bqm', ctx, w_o)

    def _B_ref(x, w_gate, w_up, w_down):
        g = jnp.einsum('bsd,df->bsf', x, w_gate)
        u = jnp.einsum('bsd,df->bsf', x, w_up)
        h = _gelu(g) * u
        return jnp.einsum('bsf,fd->bsd', h, w_down)
    x = A_x
    mod = (_silu(c) @ w_mod).reshape(c.shape[0], 6, 1, -1)
    sa, ca, ga, sb, cb, gb = (mod[:, 0].copy(), mod[:, 1].copy(), mod[:, 2].copy(), mod[:, 3].copy(), mod[:, 4].copy(), mod[:, 5].copy())
    h = _layernorm(x, axis=-1) * (1 + ca) + sa
    x = x + ga * _A_ref(h, A_c_kv, A_w_q, A_w_uk, A_w_uv, A_w_o)
    h = _layernorm(x, axis=-1) * (1 + cb) + sb
    x = x + gb * _B_ref(h, B_w_gate, B_w_up, B_w_down)
    return x
```

```python
import jax
import jax.numpy as jnp
import numpy as np
from jax.experimental import pallas as pl
from jax.experimental.pallas import tpu as pltpu

H = 32
D = 128
M = 512
F = 1792
SK = 32768

KV_DMA = 4096
KV_CH = 1024
WD_SPLIT = (1536, 256)

F32 = jnp.float32
BF16 = jnp.bfloat16
NT = (((1,), (1,)), ((), ()))


def _iota(shape, dim):
    return jax.lax.broadcasted_iota(jnp.int32, shape, dim)


def _layernorm(x):
    mu = jnp.mean(x, axis=-1, keepdims=True)
    xc = x - mu
    var = jnp.mean(xc * xc, axis=-1, keepdims=True)
    return xc * jax.lax.rsqrt(var + 1e-5)


def _stack4(v):
    return jnp.concatenate([v[:, 128 * i:128 * (i + 1)] for i in range(4)], axis=0)


def _unstack4(v):
    return jnp.concatenate([v[32 * i:32 * (i + 1), :] for i in range(4)], axis=1)


def _w_tiles(w_ref, jj):
    return [w_ref[pl.ds(pl.multiple_of((32 * i + jj) * 128, 128), 128), :] for i in range(4)]


def _headwise_matvec(v, w_ref, r_ref):
    v4 = _stack4(v).astype(BF16)
    diag = (_iota((128, 128), 0) & 31) == (_iota((128, 128), 1) & 31)

    def body(jj, acc):
        e = jnp.dot(v4, r_ref[jj], preferred_element_type=F32)
        e = jnp.where(diag, e, 0.0).astype(BF16)
        lhs = _unstack4(e)
        rhs = jnp.concatenate(_w_tiles(w_ref, jj), axis=0)
        return acc + jnp.dot(lhs, rhs, preferred_element_type=F32)

    return jax.lax.fori_loop(0, 32, body, jnp.zeros((H, D), F32), unroll=4)


def _absorb_q(q, w_ref, r_ref):
    qb = q.astype(BF16)
    diag = (_iota((128, 128), 0) & 31) == (_iota((128, 128), 1) & 31)

    def body(jj, acc):
        w = jnp.concatenate(_w_tiles(w_ref, jj), axis=0)
        t = jax.lax.dot_general(qb, w, NT, preferred_element_type=F32)
        t = jnp.where(diag, _stack4(t), 0.0).astype(BF16)
        return acc + jax.lax.dot_general(t, r_ref[jj], NT, preferred_element_type=F32)

    acc = jax.lax.fori_loop(0, 32, body, jnp.zeros((128, 128), F32), unroll=4)
    return _unstack4(acc)


def _kernel(x_hbm, c_hbm, wmod_hbm, wq_hbm, wuk_hbm, ckv_hbm, wuv_hbm, wo_hbm,
            wg_hbm, wu_hbm, wd_hbm, out_ref,
            x_v, c_v, wmod_v, wq_v, wuk_v, ckv_v, wuv_v, wo_v, wg_v, wu_v, wd_v,
            r_v, mod_v, sems):
    n_kv = SK // KV_DMA
    sem_idx = [0]

    def copy(src, dst):
        cp = pltpu.make_async_copy(src, dst, sems.at[sem_idx[0]])
        sem_idx[0] += 1
        return cp

    cp_c = copy(c_hbm, c_v)
    cp_x = copy(x_hbm, x_v)
    cp_wmod = copy(wmod_hbm, wmod_v)
    cp_wq = copy(wq_hbm, wq_v)
    cp_wuk = copy(wuk_hbm, wuk_v)
    kv_sem0 = sem_idx[0]
    cp_kv = [copy(ckv_hbm.at[pl.ds(i * KV_DMA, KV_DMA)], ckv_v.at[pl.ds(i * KV_DMA, KV_DMA)])
             for i in range(n_kv)]
    cp_wuv = copy(wuv_hbm, wuv_v)
    cp_wo = copy(wo_hbm, wo_v)
    cp_wg = copy(wg_hbm, wg_v)
    cp_wu = copy(wu_hbm, wu_v)
    cp_wd, off = [], 0
    for n in WD_SPLIT:
        cp_wd.append((copy(wd_hbm.at[pl.ds(off, n)], wd_v.at[pl.ds(off, n)]), off, n))
        off += n
    for cp in [cp_c, cp_x, cp_wmod, cp_wq, cp_wuk] + cp_kv + [cp_wuv, cp_wo, cp_wg, cp_wu] + [
            t[0] for t in cp_wd]:
        cp.start()

    dsel = _iota((128, 128), 0) - (_iota((128, 128), 1) >> 5)

    def make_r(jj, carry):
        r_v[jj] = jnp.where(dsel == 4 * jj, 1.0, 0.0).astype(BF16)
        return carry

    jax.lax.fori_loop(0, 32, make_r, 0, unroll=2)

    cp_c.wait()
    cp_x.wait()
    cf = jnp.broadcast_to(c_v[...].astype(F32), (16, M))
    sc = (cf * jax.nn.sigmoid(cf)).astype(BF16)
    x0 = jnp.broadcast_to(x_v[0].astype(F32), (16, M))
    ln0 = _layernorm(x0)
    cp_wmod.wait()
    mod = jnp.dot(sc, wmod_v[...], preferred_element_type=F32).astype(BF16).astype(F32)
    mod_v[...] = mod
    h = (ln0 * (1.0 + mod[:, M:2 * M]) + mod[:, 0:M])
    h = jnp.concatenate([h, h], axis=0)

    cp_wq.wait()
    q = _headwise_matvec(h, wq_v, r_v)
    cp_wuk.wait()
    qa = _absorb_q(q, wuk_v, r_v)
    qa = (qa * (D ** -0.5)).astype(BF16)

    per_dma = KV_DMA // KV_CH

    def kv_step(t, carry):
        m_i, l_i, acc = carry
        kv = ckv_v[pl.ds(pl.multiple_of(t * KV_CH, KV_CH), KV_CH), :]
        s = jax.lax.dot_general(qa, kv, NT, preferred_element_type=F32)
        m_new = jnp.maximum(m_i, jnp.max(s, axis=1, keepdims=True))
        alpha = jnp.exp(m_i - m_new)
        p = jnp.exp(s - m_new)
        l_new = alpha * l_i + jnp.sum(p, axis=1, keepdims=True)
        acc = alpha * acc + jnp.dot(p.astype(BF16), kv, preferred_element_type=F32)
        return m_new, l_new, acc

    def dma_step(i, carry):
        pltpu.make_async_copy(
            ckv_hbm.at[pl.ds(i * KV_DMA, KV_DMA)], ckv_v.at[pl.ds(i * KV_DMA, KV_DMA)],
            sems.at[kv_sem0 + i]).wait()
        for u in range(per_dma):
            carry = kv_step(i * per_dma + u, carry)
        return carry

    init = (jnp.full((H, 1), -jnp.inf, F32), jnp.zeros((H, 1), F32), jnp.zeros((H, M), F32))
    _, l_f, acc = jax.lax.fori_loop(0, n_kv, dma_step, init)
    o_lat = acc / l_f

    cp_wuv.wait()
    ctx = _headwise_matvec(o_lat, wuv_v, r_v)
    ctxb = ctx.astype(BF16).astype(F32)
    row16 = _iota((16, D), 0)
    bd = jnp.concatenate(
        [jnp.where(row16 == (hh % 16), ctxb[16 * (hh // 16):16 * (hh // 16) + 16, :], 0.0)
         for hh in range(H)], axis=1).astype(BF16)
    cp_wo.wait()
    attn = jnp.dot(bd, wo_v[...], preferred_element_type=F32)
    attn = jnp.sum(attn, axis=0, keepdims=True)
    attn = jnp.broadcast_to(attn, (16, M))

    mod = mod_v[...]
    x1 = x0 + mod[:, 2 * M:3 * M] * attn
    h2 = (_layernorm(x1) * (1.0 + mod[:, 4 * M:5 * M]) + mod[:, 3 * M:4 * M]).astype(BF16)
    cp_wg.wait()
    g = jnp.dot(h2, wg_v[...], preferred_element_type=F32)
    cp_wu.wait()
    u = jnp.dot(h2, wu_v[...], preferred_element_type=F32)
    gl = 0.5 * g * (1.0 + jnp.tanh(0.7978845608028654 * (g + 0.044715 * (g * g * g))))
    a = (gl * u).astype(BF16)
    y = jnp.zeros((16, M), F32)
    for cp, off, n in cp_wd:
        cp.wait()
        y = y + jnp.dot(a[:, off:off + n], wd_v[off:off + n, :], preferred_element_type=F32)
    res = x1 + mod[:, 5 * M:6 * M] * y
    out_ref[0] = res[0:1, :].astype(out_ref.dtype)


@jax.jit
def pallas_adaLN_cond__compressed_kv_cla__glu_gated_geglu__decode_kernel(
    A_x: jax.Array,
    A_c_kv: jax.Array,
    A_w_q: jax.Array,
    A_w_uk: jax.Array,
    A_w_uv: jax.Array,
    A_w_o: jax.Array,
    B_x: jax.Array,
    B_w_gate: jax.Array,
    B_w_up: jax.Array,
    B_w_down: jax.Array,
    c: jax.Array,
    w_mod: jax.Array,
):
    del B_x
    n_sems = 5 + SK // KV_DMA + 4 + len(WD_SPLIT)
    any_spec = pl.BlockSpec(memory_space=pl.ANY)
    return pl.pallas_call(
        _kernel,
        out_shape=jax.ShapeDtypeStruct((1, 1, M), A_x.dtype),
        in_specs=[any_spec] * 11,
        out_specs=pl.BlockSpec(memory_space=pltpu.VMEM),
        scratch_shapes=[
            pltpu.VMEM((1, 1, M), BF16),
            pltpu.VMEM((1, M), BF16),
            pltpu.VMEM((M, 6 * M), BF16),
            pltpu.VMEM((M * H, D), BF16),
            pltpu.VMEM((M * H, D), BF16),
            pltpu.VMEM((SK, M), BF16),
            pltpu.VMEM((M * H, D), BF16),
            pltpu.VMEM((H * D, M), BF16),
            pltpu.VMEM((M, F), BF16),
            pltpu.VMEM((M, F), BF16),
            pltpu.VMEM((F, M), BF16),
            pltpu.VMEM((32, 128, 128), BF16),
            pltpu.VMEM((16, 6 * M), F32),
            pltpu.SemaphoreType.DMA((n_sems,)),
        ],
        compiler_params=pltpu.CompilerParams(vmem_limit_bytes=100 * 1024 * 1024),
    )(
        A_x,
        c,
        w_mod,
        A_w_q.reshape(M * H, D),
        A_w_uk.reshape(M * H, D),
        A_c_kv.reshape(SK, M),
        A_w_uv.reshape(M * H, D),
        A_w_o.reshape(H * D, M),
        B_w_gate,
        B_w_up,
        B_w_down,
    )
```

```python
import jax
import jax.numpy as jnp
from jax.experimental import pallas as pl
from jax.experimental.pallas import tpu as pltpu

H = 32
D = 128
M = 512
F = 1792
SK = 32768

KV_SPLIT = (20480, 12288)
KV_CH = 2048
KV_UNROLL = 2
WD_SPLIT = (1024, 512, 256)

F32 = jnp.float32
BF16 = jnp.bfloat16
NT = (((1,), (1,)), ((), ()))


def _iota(shape, dim):
    return jax.lax.broadcasted_iota(jnp.int32, shape, dim)


def _layernorm(x):
    mu = jnp.mean(x, axis=-1, keepdims=True)
    xc = x - mu
    var = jnp.mean(xc * xc, axis=-1, keepdims=True)
    return xc * jax.lax.rsqrt(var + 1e-5)


def _stack4(v):
    return jnp.concatenate([v[:, 128 * i:128 * (i + 1)] for i in range(4)], axis=0)


def _unstack4(v):
    return jnp.concatenate([v[32 * i:32 * (i + 1), :] for i in range(4)], axis=1)


def _w_tiles(w_ref, jj):
    return [w_ref[pl.ds(pl.multiple_of((32 * i + jj) * 128, 128), 128), :] for i in range(4)]


def _headwise_matvec(v, w_ref, r_ref):
    v4 = _stack4(v).astype(BF16)
    diag = (_iota((128, 128), 0) & 31) == (_iota((128, 128), 1) & 31)

    def body(jj, acc):
        e = jnp.dot(v4, r_ref[jj], preferred_element_type=F32)
        e = jnp.where(diag, e, 0.0).astype(BF16)
        lhs = _unstack4(e)
        rhs = jnp.concatenate(_w_tiles(w_ref, jj), axis=0)
        return acc + jnp.dot(lhs, rhs, preferred_element_type=F32)

    return jax.lax.fori_loop(0, 32, body, jnp.zeros((H, D), F32), unroll=4)


def _absorb_q(q, w_ref, r_ref):
    qb = q.astype(BF16)
    diag = (_iota((128, 128), 0) & 31) == (_iota((128, 128), 1) & 31)

    def body(jj, acc):
        w = jnp.concatenate(_w_tiles(w_ref, jj), axis=0)
        t = jax.lax.dot_general(qb, w, NT, preferred_element_type=F32)
        t = jnp.where(diag, _stack4(t), 0.0).astype(BF16)
        return acc + jax.lax.dot_general(t, r_ref[jj], NT, preferred_element_type=F32)

    acc = jax.lax.fori_loop(0, 32, body, jnp.zeros((128, 128), F32), unroll=4)
    return _unstack4(acc)


def _kernel(x_hbm, c_hbm, wmod_hbm, wq_hbm, wuk_hbm, ckv_hbm, wuv_hbm, wo_hbm,
            wg_hbm, wu_hbm, wd_hbm, out_ref,
            x_v, c_v, wmod_v, wq_v, wuk_v, ckv_v, wuv_v, wo_v, wg_v, wu_v, wd_v,
            r_v, mod_v, a_v, sems):
    sem_idx = [0]

    def copy(src, dst):
        cp = pltpu.make_async_copy(src, dst, sems.at[sem_idx[0]])
        sem_idx[0] += 1
        return cp

    def pieces(src, dst, split):
        out, off = [], 0
        for n in split:
            out.append((copy(src.at[pl.ds(off, n)], dst.at[pl.ds(off, n)]), off, n))
            off += n
        return out

    cp_c = copy(c_hbm, c_v)
    cp_x = copy(x_hbm, x_v)
    cp_wmod = copy(wmod_hbm, wmod_v)
    cp_wq = copy(wq_hbm, wq_v)
    cp_wuk = copy(wuk_hbm, wuk_v)
    cp_kv = pieces(ckv_hbm, ckv_v, KV_SPLIT)
    cp_wuv = copy(wuv_hbm, wuv_v)
    cp_wo = copy(wo_hbm, wo_v)
    cp_wg = copy(wg_hbm, wg_v)
    cp_wu = copy(wu_hbm, wu_v)
    cp_wd = pieces(wd_hbm, wd_v, WD_SPLIT)
    for cp in ([cp_c, cp_x, cp_wmod, cp_wq, cp_wuk] + [t[0] for t in cp_kv]
               + [cp_wuv, cp_wo, cp_wg, cp_wu] + [t[0] for t in cp_wd]):
        cp.start()

    dsel = _iota((128, 128), 0) - (_iota((128, 128), 1) >> 5)

    def make_r(jj, carry):
        r_v[jj] = jnp.where(dsel == 4 * jj, 1.0, 0.0).astype(BF16)
        return carry

    jax.lax.fori_loop(0, 32, make_r, 0, unroll=2)

    cp_c.wait()
    cp_x.wait()
    cf = jnp.broadcast_to(c_v[...].astype(F32), (16, M))
    sc = (cf * jax.nn.sigmoid(cf)).astype(BF16)
    x0 = jnp.broadcast_to(x_v[0].astype(F32), (16, M))
    ln0 = _layernorm(x0)
    cp_wmod.wait()
    mod = jnp.dot(sc, wmod_v[...], preferred_element_type=F32).astype(BF16).astype(F32)
    mod_v[...] = mod
    h = (ln0 * (1.0 + mod[:, M:2 * M]) + mod[:, 0:M])
    h = jnp.concatenate([h, h], axis=0)

    cp_wq.wait()
    q = _headwise_matvec(h, wq_v, r_v)
    cp_wuk.wait()
    qa = _absorb_q(q, wuk_v, r_v)
    qa = (qa * (D ** -0.5)).astype(BF16)

    def kv_step(t, carry):
        m_i, l_i, acc = carry
        kv = ckv_v[pl.ds(pl.multiple_of(t * KV_CH, KV_CH), KV_CH), :]
        s = jax.lax.dot_general(qa, kv, NT, preferred_element_type=F32)
        m_new = jnp.maximum(m_i, jnp.max(s, axis=1, keepdims=True))
        alpha = jnp.exp(m_i - m_new)
        p = jnp.exp(s - m_new)
        l_new = alpha * l_i + jnp.sum(p, axis=1, keepdims=True)
        acc = alpha * acc + jnp.dot(p.astype(BF16), kv, preferred_element_type=F32)
        return m_new, l_new, acc

    carry = (jnp.full((H, 1), -jnp.inf, F32), jnp.zeros((H, 1), F32), jnp.zeros((H, M), F32))
    for cp, off, n in cp_kv:
        cp.wait()
        carry = jax.lax.fori_loop(off // KV_CH, (off + n) // KV_CH, kv_step, carry,
                                  unroll=KV_UNROLL)
    _, l_f, acc = carry
    o_lat = acc / l_f

    cp_wuv.wait()
    ctx = _headwise_matvec(o_lat, wuv_v, r_v)
    ctxb = ctx.astype(BF16).astype(F32)
    row16 = _iota((16, D), 0)
    bd = jnp.concatenate(
        [jnp.where(row16 == (hh % 16), ctxb[16 * (hh // 16):16 * (hh // 16) + 16, :], 0.0)
         for hh in range(H)], axis=1).astype(BF16)
    cp_wo.wait()
    attn = jnp.dot(bd, wo_v[...], preferred_element_type=F32)
    attn = jnp.sum(attn, axis=0, keepdims=True)
    attn = jnp.broadcast_to(attn, (16, M))

    mod = mod_v[...]
    x1 = x0 + mod[:, 2 * M:3 * M] * attn
    h2 = (_layernorm(x1) * (1.0 + mod[:, 4 * M:5 * M]) + mod[:, 3 * M:4 * M]).astype(BF16)
    cp_wg.wait()
    g = jnp.dot(h2, wg_v[...], preferred_element_type=F32)
    cp_wu.wait()
    u = jnp.dot(h2, wu_v[...], preferred_element_type=F32)
    gl = 0.5 * g * (1.0 + jnp.tanh(0.7978845608028654 * (g + 0.044715 * (g * g * g))))
    a = (gl * u).astype(BF16)
    a_v[...] = a

    def wd_dot(off, n, y):
        return y + jnp.dot(a_v[:, pl.ds(off, n)], wd_v[pl.ds(off, n), :],
                           preferred_element_type=F32)

    y = jnp.zeros((16, M), F32)
    for k, (cp, off, n) in enumerate(cp_wd):
        cp.wait()
        if k == len(cp_wd) - 1:
            y = wd_dot(off, n, y)
        else:
            half = n // 2
            y = jax.lax.fori_loop(
                0, 2,
                lambda i, y, off=off, half=half: wd_dot(
                    pl.multiple_of(off + i * half, 128), half, y), y)
    res = x1 + mod[:, 5 * M:6 * M] * y
    out_ref[0] = res[0:1, :].astype(out_ref.dtype)


@jax.jit
def pallas_adaLN_cond__compressed_kv_cla__glu_gated_geglu__decode_kernel(
    A_x: jax.Array,
    A_c_kv: jax.Array,
    A_w_q: jax.Array,
    A_w_uk: jax.Array,
    A_w_uv: jax.Array,
    A_w_o: jax.Array,
    B_x: jax.Array,
    B_w_gate: jax.Array,
    B_w_up: jax.Array,
    B_w_down: jax.Array,
    c: jax.Array,
    w_mod: jax.Array,
):
    del B_x
    n_sems = 9 + len(KV_SPLIT) + len(WD_SPLIT)
    any_spec = pl.BlockSpec(memory_space=pl.ANY)
    return pl.pallas_call(
        _kernel,
        out_shape=jax.ShapeDtypeStruct((1, 1, M), A_x.dtype),
        in_specs=[any_spec] * 11,
        out_specs=pl.BlockSpec(memory_space=pltpu.VMEM),
        scratch_shapes=[
            pltpu.VMEM((1, 1, M), BF16),
            pltpu.VMEM((1, M), BF16),
            pltpu.VMEM((M, 6 * M), BF16),
            pltpu.VMEM((M * H, D), BF16),
            pltpu.VMEM((M * H, D), BF16),
            pltpu.VMEM((SK, M), BF16),
            pltpu.VMEM((M * H, D), BF16),
            pltpu.VMEM((H * D, M), BF16),
            pltpu.VMEM((M, F), BF16),
            pltpu.VMEM((M, F), BF16),
            pltpu.VMEM((F, M), BF16),
            pltpu.VMEM((32, 128, 128), BF16),
            pltpu.VMEM((16, 6 * M), F32),
            pltpu.VMEM((16, F), BF16),
            pltpu.SemaphoreType.DMA((n_sems,)),
        ],
        compiler_params=pltpu.CompilerParams(vmem_limit_bytes=100 * 1024 * 1024),
    )(
        A_x,
        c,
        w_mod,
        A_w_q.reshape(M * H, D),
        A_w_uk.reshape(M * H, D),
        A_c_kv.reshape(SK, M),
        A_w_uv.reshape(M * H, D),
        A_w_o.reshape(H * D, M),
        B_w_gate,
        B_w_up,
        B_w_down,
    )
```
